```python
import os as _os
_os.environ.setdefault("JAX_PLATFORMS", "cpu")
import jax
import jax.numpy as jnp

def _softmax(x, axis=-1):
    return jax.nn.softmax(x, axis=axis)
def _gelu(x):
    return jax.nn.gelu(x, approximate=True)
def _silu(x):
    return jax.nn.silu(x)
def _sigmoid(x):
    return jax.nn.sigmoid(x)
def _layernorm(x, axis=-1, eps=1e-5):
    m = jnp.mean(x, axis=axis, keepdims=True)
    v = jnp.var(x, axis=axis, keepdims=True)
    return (x - m) / jnp.sqrt(v + eps)
def _scatter_add(tgt, idx, src, axis=0):
    return tgt.at[idx].add(src)
def _segment_sum(src, seg, n):
    return jax.ops.segment_sum(src, seg, n)
class _Rng:
    def __init__(self, key):
        self._k = key
    def _next(self):
        self._k, sub = jax.random.split(self._k)
        return sub
    def normal(self, shape):
        return jax.random.normal(self._next(), shape, dtype=jnp.bfloat16)
    def randint(self, lo, hi, shape):
        return jax.random.randint(self._next(), shape, lo, hi, dtype=jnp.int32)
    def uniform(self, shape, lo=0.0, hi=1.0):
        return jax.random.uniform(self._next(), shape, jnp.bfloat16, lo, hi)
    def permutation(self, n):
        return jax.random.permutation(self._next(), n)


kernel_name = 'standalone__sliding_block_cached__sampling'

def setup_inputs():
    _rng = _Rng(jax.random.key(int.from_bytes(__import__("os").urandom(4), "little")))
    _w = (lambda a: (lambda t: t.astype(jnp.bfloat16) if jnp.issubdtype(t.dtype, jnp.floating) else t)(jnp.asarray(a)))
    B, Sq, D = 8, 4, 640
    Hq, Hkv, Sk, Dh = 32, 32, 4096, 192
    assert Hq % Hkv == 0, (Hq, Hkv)
    return {
        "x": _w((lambda *s: _rng.normal(s) * 0.8)(B, Sq, D)),
        "k_cache": _w((lambda *s: _rng.normal(s) * 0.8)(B, Hkv, Sk, Dh)),
        "v_cache": _w((lambda *s: _rng.normal(s) * 0.05)(B, Hkv, Sk, Dh)),
        "wq": _w((lambda *s: _rng.normal(s) * 0.8)(D, Hq * Dh) * (D ** -0.5)),
        "wo": _w((lambda *s: _rng.normal(s) * 0.05)(Hq * Dh, D) * ((Hq * Dh) ** -0.5)),
    }

def reference(x, k_cache, v_cache, wq, wo):
    B, Sq, D = x.shape
    Hq, Dh = 32, 192
    Hkv, Sk = k_cache.shape[1], k_cache.shape[2]
    W = min(4096, max(256, Sk // 4))
    rep = Hq // Hkv
    q = (lambda x, *d: x.transpose(*d))((x @ wq).reshape(B, Sq, Hq, Dh), 0, 2, 1, 3)
    k = jnp.repeat(k_cache[:, :, Sk - W:, :], rep, axis=1)
    v = jnp.repeat(v_cache[:, :, Sk - W:, :], rep, axis=1)
    scores = jnp.einsum("bhqd,bhkd->bhqk", q, k) * (Dh ** -0.5)
    p = _softmax(scores, axis=-1)
    o = jnp.einsum("bhqk,bhkd->bhqd", p, v)
    return (lambda x, *d: x.transpose(*d))(o, 0, 2, 1, 3).reshape(B, Sq, Hq * Dh) @ wo
```

```python
import functools
import jax, jax.numpy as jnp
from jax import lax
from jax.experimental import pallas as pl
from jax.experimental.pallas import tpu as pltpu

B, SQ, D = 8, 4, 640
H, SK, DH = 32, 4096, 192
W = 1024
NU = H * (B // 2)
NSTEP = 9

def make(LA=45, skew=28, NS=None, compute=True, nobounds=True):
    LB = LA
    LAa = LA - skew
    assert LAa >= 1
    ns = NS or (-(-LB // NSTEP) + 1)
    scale = DH ** -0.5

    def kernel(x_hbm, k_hbm, v_hbm, wq_hbm, wo_hbm, o_ref,
               kv, wq_v, wo_v, x_v, x32, q_scr, o_scr, acc, semA, semB, sem0):
        def piece(u, j, qi):
            sem = (semA if qi == 0 else semB).at[lax.rem(u, ns), j]
            slot = lax.rem(u, ns)
            h = u // 4
            bp = lax.rem(u, 4)
            if j == 4:
                hp = u // 8
                part = lax.rem(u, 8)
                if qi == 0:
                    r = pl.multiple_of(hp * 384 + part * 48, 16)
                    return pltpu.make_async_copy(wo_hbm.at[pl.ds(r, 48), :], wo_v.at[pl.ds(r, 48), :], sem)
                else:
                    r = pl.multiple_of(part * 80, 16)
                    c = pl.multiple_of((hp + 1) * 384, 128)
                    return pltpu.make_async_copy(wq_hbm.at[pl.ds(r, 80), pl.ds(c, 384)], wq_v.at[hp + 1, pl.ds(r, 80), :], sem)
            jj = j if j < 4 else j - 5
            src = k_hbm if j < 4 else v_hbm
            t = (0 if j < 4 else 2) + jj // 2
            b = 2 * bp + jj // 2
            c = (jj % 2) * 512 + (256 if qi == 0 else 0)
            row = pl.multiple_of((b * H + h) * DH, DH)
            return pltpu.make_async_copy(src.at[pl.ds(row, DH), pl.ds(SK - W + c, 256)],
                                         kv.at[slot, t, :, pl.ds(c, 256)], sem)

        def exists(u, j, qi):
            if j == 4 and qi == 1:
                return u < NU - 8
            return u < NU

        def start(u, j, qi):
            if isinstance(u, int):
                if exists(u, j, qi):
                    piece(jnp.int32(u), j, qi).start(priority=qi)
            else:
                @pl.when(exists(u, j, qi))
                def _():
                    piece(u, j, qi).start(priority=qi)

        def wait(u, j, qi):
            if j == 4 and qi == 1:
                @pl.when(exists(u, j, qi))
                def _():
                    piece(u, j, qi).wait()
            else:
                piece(u, j, qi).wait()

        cx = pltpu.make_async_copy(x_hbm, x_v, sem0.at[0])
        cw0 = pltpu.make_async_copy(wq_hbm.at[pl.ds(0, 320), pl.ds(0, 384)], wq_v.at[0, pl.ds(0, 320), :], sem0.at[1])
        cw1 = pltpu.make_async_copy(wq_hbm.at[pl.ds(320, 320), pl.ds(0, 384)], wq_v.at[0, pl.ds(320, 320), :], sem0.at[2])
        cw1.start(priority=1)
        cx.start(priority=0)
        cw0.start(priority=0)
        for s in range(LB):
            start(s // NSTEP, s % NSTEP, 1)
            sa = s - skew
            if sa >= 0:
                start(sa // NSTEP, sa % NSTEP, 0)
        cx.wait()
        for b in range(B):
            x32[pl.ds(4 * b, 4), :] = x_v[b].astype(jnp.float32)
        acc[...] = jnp.zeros_like(acc)
        cw0.wait()
        cw1.wait()

        row_lo = lax.broadcasted_iota(jnp.int32, (8, 1), 0) < 4

        def body(u, carry):
            slot = lax.rem(u, ns)
            h = u // 4
            bp = lax.rem(u, 4)

            def dma_step(j):
                sb = j + LB
                start(u + sb // NSTEP, sb % NSTEP, 1)
                sa = j + LAa
                start(u + sa // NSTEP, sa % NSTEP, 0)
                wait(u, j, 1)
                wait(u, j, 0)

            @pl.when(lax.rem(u, 8) == 0)
            def _():
                qp = jnp.dot(x32[...].astype(jnp.bfloat16), wq_v[u // 8], preferred_element_type=jnp.float32)
                q_scr[0] = qp[:, :DH]
                q_scr[1] = qp[:, DH:]

            if not compute:
                for j in range(NSTEP):
                    dma_step(j)
                return carry

            q8 = q_scr[lax.rem(h, 2), pl.ds(pl.multiple_of(bp * 8, 8), 8), :].astype(jnp.bfloat16)
            s_parts = []
            for j in range(4):
                dma_step(j)
                kt = kv[slot, j // 2, :, pl.ds((j % 2) * 512, 512)]
                s_parts.append(jnp.dot(q8, kt, preferred_element_type=jnp.float32))
            dma_step(4)
            s0 = jnp.where(row_lo, s_parts[0], s_parts[2]) * scale
            s1 = jnp.where(row_lo, s_parts[1], s_parts[3]) * scale
            m = jnp.maximum(jnp.max(s0, axis=1, keepdims=True), jnp.max(s1, axis=1, keepdims=True))
            p0 = jnp.exp(s0 - m)
            p1 = jnp.exp(s1 - m)
            l = jnp.sum(p0, axis=1, keepdims=True) + jnp.sum(p1, axis=1, keepdims=True)
            pb = [p0.astype(jnp.bfloat16), p1.astype(jnp.bfloat16)]
            o_parts = []
            for j in range(4):
                dma_step(5 + j)
                vt = kv[slot, 2 + j // 2, :, pl.ds((j % 2) * 512, 512)]
                o_parts.append(lax.dot_general(pb[j % 2], vt, (((1,), (1,)), ((), ())), preferred_element_type=jnp.float32))
            o = jnp.where(row_lo, o_parts[0] + o_parts[1], o_parts[2] + o_parts[3]) / l
            o_scr[pl.ds(pl.multiple_of(bp * 8, 8), 8), :] = o

            @pl.when(bp == 3)
            def _():
                r = pl.multiple_of(h * DH, 16)
                acc[...] += jnp.dot(o_scr[...].astype(jnp.bfloat16), wo_v[pl.ds(r, DH), :], preferred_element_type=jnp.float32)
            return carry

        lax.fori_loop(0, NU, body, 0)
        for b in range(B):
            o_ref[b] = acc[pl.ds(4 * b, 4), :].astype(o_ref.dtype)

    def fn(x, k_cache, v_cache, wq, wo):
        kt = jnp.swapaxes(k_cache, 2, 3).reshape(B * H * DH, SK)
        vt = jnp.swapaxes(v_cache, 2, 3).reshape(B * H * DH, SK)
        any_spec = pl.BlockSpec(memory_space=pl.ANY)
        return pl.pallas_call(
            kernel,
            in_specs=[any_spec] * 5,
            out_specs=pl.BlockSpec(memory_space=pltpu.VMEM),
            out_shape=jax.ShapeDtypeStruct((B, SQ, D), jnp.bfloat16),
            scratch_shapes=[
                pltpu.VMEM((ns, 4, DH, W), jnp.bfloat16),
                pltpu.VMEM((H // 2, D, 2 * DH), jnp.bfloat16),
                pltpu.VMEM((H * DH, D), jnp.bfloat16),
                pltpu.VMEM((B, SQ, D), jnp.bfloat16),
                pltpu.VMEM((B * SQ, D), jnp.float32),
                pltpu.VMEM((2, B * SQ, DH), jnp.float32),
                pltpu.VMEM((B * SQ, DH), jnp.float32),
                pltpu.VMEM((B * SQ, D), jnp.float32),
                pltpu.SemaphoreType.DMA((ns, NSTEP)),
                pltpu.SemaphoreType.DMA((ns, NSTEP)),
                pltpu.SemaphoreType.DMA((3,)),
            ],
            compiler_params=pltpu.CompilerParams(vmem_limit_bytes=100 * 1024 * 1024, disable_bounds_checks=nobounds),
        )(x, kt, vt, wq, wo)
    return fn


@jax.jit
def pallas_standalone__sliding_block_cached__sampling_kernel(x, k_cache, v_cache, wq, wo):
    return make()(x, k_cache, v_cache, wq, wo)
```

```python
import functools
import numpy as np
import jax, jax.numpy as jnp
from jax import lax
from jax.experimental import pallas as pl
from jax.experimental.pallas import tpu as pltpu

B, SQ, D = 8, 4, 640
H, SK, DH = 32, 4096, 192
W = 1024
NU = H * (B // 2)
PR = 16
NT_DIMS = (((1,), (1,)), ((), ()))

def make(LA=2, order="wjg", tail=2, wo_rows=24, compute=True, wq_mode=0, wo_mode=0):
    LB = LA + 1
    ns = LB + 1
    scale = DH ** -0.5
    import itertools
    dims = {'w': [0, 1], 'j': [0, 1], 'g': [0, 1, 2]}
    regs = [dict(zip(order, c)) for c in itertools.product(*[dims[k] for k in order])]
    ps = [(r['w'], r['j'], r['g'] * 64 + s * PR) for s in range(4) for r in regs]
    PB, PA = ps[0::2], ps[1::2]
    last = [(0, j, g * 64 + s * PR, 0) for s in range(4) for j in range(2) for g in range(3)]
    last += [(1, 0, g * 64 + s * PR, 1) for s in range(4) for g in range(3)]
    last += [(1, 1, g * 64 + s * PR, 2) for s in range(4) for g in range(2)]
    last += [(1, 1, 128 + s * PR, 3) for s in range(4)]
    n_wq = 240
    n_wo = (H * DH) // wo_rows
    n_wo_pairs = (n_wo - len(PB)) // 2

    def kernel(x_hbm, k_hbm, v_hbm, wq_hbm, wo_hbm, o_ref,
               kv, wq_v, wo_v, x_v, x32, q_scr, o_scr, acc, sems, sem0, seml):
        def kv_copy(u, slot, w, j, r, sem):
            row0 = (2 * lax.rem(u, 4) * H + u // 4) * DH
            src = k_hbm if w == 0 else v_hbm
            row = pl.multiple_of(row0 + (j * H * DH + r), PR)
            return pltpu.make_async_copy(src.at[pl.ds(row, PR), pl.ds(SK - W, W)],
                                         kv.at[slot, 2 * w + j, pl.ds(r, PR), :], sem)

        def wq_copy(k):
            if wq_mode == 0:
                idx = lax.rem(k, 15) * 16 + k // 15
            else:
                idx = lax.rem(k * 97, n_wq)
            r = pl.multiple_of((idx // 3) * 8, 8)
            c = pl.multiple_of(lax.rem(idx, 3) * 2048, 2048)
            return pltpu.make_async_copy(wq_hbm.at[pl.ds(r, 8), pl.ds(c, 2048)], wq_v.at[pl.ds(r, 8), pl.ds(c, 2048)], sem0.at[1])

        def wo_copy(k):
            if wo_mode == 0:
                idx = lax.rem(k, 16) * (n_wo // 16) + k // 16
            else:
                idx = lax.rem(k * 101, n_wo)
            r = pl.multiple_of(idx * wo_rows, 8)
            return pltpu.make_async_copy(wo_hbm.at[pl.ds(r, wo_rows), :], wo_v.at[pl.ds(r, wo_rows), :], sem0.at[2])

        cx = pltpu.make_async_copy(x_hbm, x_v, sem0.at[0])
        cx.start()

        def wq_body(i, c):
            wq_copy(2 * i).start(priority=1)
            wq_copy(2 * i + 1).start(priority=0)
            return c
        lax.fori_loop(0, n_wq // 2, wq_body, 0)

        def wo_body(i, c):
            wo_copy(2 * i).start(priority=1)
            wo_copy(2 * i + 1).start(priority=0)
            return c

        cx.wait()
        for b in range(B):
            x32[pl.ds(4 * b, 4), :] = x_v[b].astype(jnp.float32)
        acc[...] = jnp.zeros_like(acc)

        NQ = H // 2
        n_first = 36
        lax.fori_loop(0, n_first, wo_body, 0)
        pltpu.make_async_copy(wq_v, wq_v, sem0.at[1]).wait()
        per = -(-(n_wo_pairs - n_first) // NQ)

        def q_body(hp, c):
            lo = n_first + hp * per
            lax.fori_loop(lo, jnp.minimum(lo + per, n_wo_pairs), wo_body, 0)
            col = pl.multiple_of(hp * 2 * DH, 128)
            qp = jnp.dot(x32[...].astype(jnp.bfloat16), wq_v[:, pl.ds(col, 2 * DH)], preferred_element_type=jnp.float32)
            q_scr[2 * hp] = qp[:, :DH]
            q_scr[2 * hp + 1] = qp[:, DH:]
            return c
        lax.fori_loop(0, NQ, q_body, 0)

        for i, (w, j, r) in enumerate(PB):
            kv_copy(jnp.int32(0), 0, w, j, r, sems.at[0]).start(priority=1)
            wo_copy(jnp.int32(2 * n_wo_pairs + i)).start(priority=0)

        def issue(ua, slot_a, slot_b):
            for (wb, jb, rb), (wa, ja, ra) in zip(PB, PA):
                kv_copy(ua + 1, slot_b, wb, jb, rb, sems.at[slot_b]).start(priority=1)
                kv_copy(ua, slot_a, wa, ja, ra, sems.at[slot_a]).start(priority=0)

        def pre_body(u, c):
            issue(u, u, u + 1)
            return c
        lax.fori_loop(0, LA, pre_body, 0)
        pltpu.make_async_copy(wo_v, wo_v, sem0.at[2]).wait()

        row_lo = lax.broadcasted_iota(jnp.int32, (8, 1), 0) < 4

        def scores(u, slot):
            h = u // 4
            bp = lax.rem(u, 4)
            q8 = q_scr[h, pl.ds(pl.multiple_of(bp * 8, 8), 8), :].astype(jnp.bfloat16)
            se = jnp.dot(q8, kv[slot, 0], preferred_element_type=jnp.float32)
            so = jnp.dot(q8, kv[slot, 1], preferred_element_type=jnp.float32)
            s = jnp.where(row_lo, se, so) * scale
            m = jnp.max(s, axis=1, keepdims=True)
            p = jnp.exp(s - m)
            l = jnp.sum(p, axis=1, keepdims=True)
            return p.astype(jnp.bfloat16), l

        def wrap(s):
            return jnp.where(s >= ns, s - ns, s)

        last_slot = (NU - 1) % ns

        def body(u, slot):
            h = u // 4
            bp = lax.rem(u, 4)
            slot_a = wrap(slot + LA)
            slot_b = wrap(slot + LB)

            @pl.when(u + LB < NU - 1)
            def _():
                issue(u + LA, slot_a, slot_b)

            @pl.when(u + LB == NU - 1)
            def _():
                for i, (w, j, r, t) in enumerate(last):
                    kv_copy(jnp.int32(NU - 1), last_slot, w, j, r, seml.at[t]).start(priority=1)
                    if i < len(PA):
                        wa, ja, ra = PA[i]
                        kv_copy(jnp.int32(NU - 2), (NU - 2) % ns, wa, ja, ra, sems.at[(NU - 2) % ns]).start(priority=0)

            pltpu.make_async_copy(kv.at[slot], kv.at[slot], sems.at[slot]).wait()
            if compute:
                pb, l = scores(u, slot)
                oe = lax.dot_general(pb, kv[slot, 2], NT_DIMS, preferred_element_type=jnp.float32)
                oo = lax.dot_general(pb, kv[slot, 3], NT_DIMS, preferred_element_type=jnp.float32)
                o_scr[pl.ds(pl.multiple_of(bp * 8, 8), 8), :] = jnp.where(row_lo, oe, oo) / l

                @pl.when(bp == 3)
                def _():
                    r = pl.multiple_of(h * DH, 16)
                    acc[...] += jnp.dot(o_scr[...].astype(jnp.bfloat16), wo_v[pl.ds(r, DH), :], preferred_element_type=jnp.float32)
            return wrap(slot + 1)

        lax.fori_loop(0, NU - 1, body, jnp.int32(0))

        sl = last_slot
        def wait_part(t, ref):
            pltpu.make_async_copy(ref, ref, seml.at[t]).wait()
        r0 = (H - 1) * DH
        wait_part(0, kv.at[sl, pl.ds(0, 2)])
        pb, l = scores(jnp.int32(NU - 1), sl)
        wait_part(1, kv.at[sl, 2])
        oe = lax.dot_general(pb, kv[sl, 2], NT_DIMS, preferred_element_type=jnp.float32)
        wait_part(2, kv.at[sl, 3, pl.ds(0, 128)])
        if tail == 1:
            wait_part(3, kv.at[sl, 3, pl.ds(128, 64)])
            oo = lax.dot_general(pb, kv[sl, 3], NT_DIMS, preferred_element_type=jnp.float32)
            o_scr[pl.ds(24, 8), :] = jnp.where(row_lo, oe, oo) / l
            res = acc[...] + jnp.dot(o_scr[...].astype(jnp.bfloat16), wo_v[pl.ds(r0, DH), :], preferred_element_type=jnp.float32)
            for b in range(B):
                o_ref[b] = res[4 * b:4 * b + 4].astype(o_ref.dtype)
        else:
            oo_lo = lax.dot_general(pb, kv[sl, 3, pl.ds(0, 128), :], NT_DIMS, preferred_element_type=jnp.float32)
            o_scr[pl.ds(24, 8), pl.ds(0, 128)] = jnp.where(row_lo, oe[:, :128], oo_lo) / l
            o_scr[pl.ds(24, 8), pl.ds(128, 64)] = jnp.where(row_lo, oe[:, 128:], 0.0) / l
            res = acc[...] + jnp.dot(o_scr[...].astype(jnp.bfloat16), wo_v[pl.ds(r0, DH), :], preferred_element_type=jnp.float32)
            for b in range(B - 1):
                o_ref[b] = res[4 * b:4 * b + 4].astype(o_ref.dtype)
            res_last = res[24:32]
            wait_part(3, kv.at[sl, 3, pl.ds(128, 64)])
            oo_hi = lax.dot_general(pb, kv[sl, 3, pl.ds(128, 64), :], NT_DIMS, preferred_element_type=jnp.float32)
            o_hi = (oo_hi / l).astype(jnp.bfloat16)
            fin = res_last + jnp.dot(o_hi, wo_v[pl.ds(r0 + 128, 64), :], preferred_element_type=jnp.float32)
            o_ref[B - 1] = fin[4:8].astype(o_ref.dtype)

    def fn(x, k_cache, v_cache, wq, wo):
        kt = jnp.swapaxes(k_cache, 2, 3).reshape(B * H * DH, SK)
        vt = jnp.swapaxes(v_cache, 2, 3).reshape(B * H * DH, SK)
        any_spec = pl.BlockSpec(memory_space=pl.ANY)
        return pl.pallas_call(
            kernel,
            in_specs=[any_spec] * 5,
            out_specs=pl.BlockSpec(memory_space=pltpu.VMEM),
            out_shape=jax.ShapeDtypeStruct((B, SQ, D), jnp.bfloat16),
            scratch_shapes=[
                pltpu.VMEM((ns, 4, DH, W), jnp.bfloat16),
                pltpu.VMEM((D, H * DH), jnp.bfloat16),
                pltpu.VMEM((H * DH, D), jnp.bfloat16),
                pltpu.VMEM((B, SQ, D), jnp.bfloat16),
                pltpu.VMEM((B * SQ, D), jnp.float32),
                pltpu.VMEM((H, B * SQ, DH), jnp.float32),
                pltpu.VMEM((B * SQ, DH), jnp.float32),
                pltpu.VMEM((B * SQ, D), jnp.float32),
                pltpu.SemaphoreType.DMA((ns,)),
                pltpu.SemaphoreType.DMA((3,)),
                pltpu.SemaphoreType.DMA((4,)),
            ],
            compiler_params=pltpu.CompilerParams(vmem_limit_bytes=100 * 1024 * 1024, disable_bounds_checks=True),
        )(x, kt, vt, wq, wo)
    return fn


@jax.jit
def pallas_standalone__sliding_block_cached__sampling_kernel(x, k_cache, v_cache, wq, wo):
    return make(order="jgw")(x, k_cache, v_cache, wq, wo)
```

```python
import jax
import jax.numpy as jnp
from jax import lax
import jax.experimental.pallas as pl
import jax.experimental.pallas.tpu as pltpu

_HEADS = 32
_ROWS = 8
_REGION = 64
_PAIRS = 4
_GROUP = 2
_HALF = 24
_WQ_COLS = 1024
_WO_ROWS = 16
_WQ_SPREAD, _WO_SPREAD = 8, 6
_GRAY = (0, 1, 3, 2, 6, 7, 5, 4)
_NT = (((1,), (1,)), ((), ()))


def _dot(a, b):
    return jnp.dot(a, b, preferred_element_type=jnp.float32)


def _dot_nt(a, b):
    return lax.dot_general(a, b, _NT, preferred_element_type=jnp.float32)


@jax.jit
def pallas_standalone__sliding_block_cached__sampling_kernel(
    x: jax.Array,
    k_cache: jax.Array,
    v_cache: jax.Array,
    wq: jax.Array,
    wo: jax.Array,
):
    B, SQ, D = x.shape
    _, H, SK, DH = k_cache.shape
    W = min(4096, max(256, SK // 4))
    scale = DH**-0.5
    cdt = k_cache.dtype

    PAIR = 2 * DH
    UNIT = _PAIRS * PAIR
    NB = B * H // 2
    N_MAIN = NB - _PAIRS
    NP = 2 * _HALF
    NR = UNIT // _REGION
    assert (H, SQ, DH) == (_HEADS, 4, 3 * _REGION) and NP * _ROWS == PAIR

    regions = list(range(0, NR, 2)) + list(range(1, NR, 2))
    groups = [_ROWS * g for g in _GRAY]

    r_last = (H - 2) * DH
    n_wq_cols = H * DH // _WQ_COLS
    NQ = (D // 8) * n_wq_cols
    NO = r_last // _WO_ROWS
    NW = (NQ + NO) // 2
    assert D % 8 == 0 and n_wq_cols * _WQ_COLS == H * DH and NO * _WO_ROWS == r_last
    assert NQ % _WQ_SPREAD == 0 and NO % _WO_SPREAD == 0
    assert NW <= NQ < 2 * NW - _HALF and NQ % _GROUP == 0 and NW % _GROUP == 0

    t_last = UNIT - PAIR
    tail = [(0, t_last + r * _REGION + g, 0) for g in groups for r in range(6)]
    tail += [(1, t_last + r * _REGION + g, 1) for g in groups for r in range(3)]
    tail += [(1, t_last + r * _REGION + g, 2) for g in groups for r in range(3, 5)]
    tail += [(1, t_last + 5 * _REGION + g, 3) for g in groups]
    tail += [(None, r, 4) for r in range(r_last, r_last + DH, _WO_ROWS)]
    tail += [(None, r, 5) for r in range(r_last + DH, r_last + DH + 128, _WO_ROWS)]
    tail += [(None, r, 6) for r in range(r_last + DH + 128, H * DH, _WO_ROWS)]
    n_both = len(tail) - _HALF
    assert n_both == 2 * NP
    tail_lo = [c for i, c in enumerate(tail[:n_both]) if (i // _GROUP) % 2 == 0]
    tail_lo += tail[n_both:]
    tail_hi = [c for i, c in enumerate(tail[:n_both]) if (i // _GROUP) % 2 == 1]

    def kernel(x_hbm, k_hbm, v_hbm, wq_hbm, wo_hbm, o_ref,
               kv, wq_v, wo_v, x_v, x_dup, q_scr, o_scr, acc,
               unit_sems, head_sems, pair_sems, tail_sems):
        def kv_copy(u, which, r, sem):
            row0 = (lax.rem(u, B) * H + lax.div(u, B) * 2 * _PAIRS) * DH
            if not isinstance(r, int):
                r = pl.multiple_of(r, _ROWS)
            src = (k_hbm, v_hbm)[which]
            return pltpu.make_async_copy(
                src.at[pl.ds(pl.multiple_of(row0 + r, _ROWS), _ROWS), pl.ds(SK - W, W)],
                kv.at[lax.rem(u, 3), which, pl.ds(r, _ROWS), :],
                sem,
            )

        def block_copies(n, which, by_pair):
            u, p = lax.div(n, _PAIRS), lax.rem(n, _PAIRS)
            if by_pair:
                return lambda i: kv_copy(
                    u, which, p * PAIR + ((i % 6) * _REGION + groups[i // 6]), pair_sems.at[p])
            gs = [(s ^ (s >> 1)) * _ROWS for s in (2 * p, 2 * p + 1)]
            return lambda i: kv_copy(
                u, which, regions[i % NR] * _REGION + gs[i // NR], unit_sems.at[lax.rem(u, 3)])

        def wq_copy(k):
            idx = lax.rem(k, _WQ_SPREAD) * (NQ // _WQ_SPREAD) + lax.div(k, _WQ_SPREAD)
            r = pl.ds(pl.multiple_of(lax.div(idx, n_wq_cols) * 8, 8), 8)
            c = pl.ds(pl.multiple_of(lax.rem(idx, n_wq_cols) * _WQ_COLS, _WQ_COLS), _WQ_COLS)
            return pltpu.make_async_copy(wq_hbm.at[r, c], wq_v.at[r, c], head_sems.at[1])

        def wo_copy(k):
            idx = lax.rem(k, _WO_SPREAD) * (NO // _WO_SPREAD) + lax.div(k, _WO_SPREAD)
            r = pl.ds(pl.multiple_of(idx * _WO_ROWS, _WO_ROWS), _WO_ROWS)
            return pltpu.make_async_copy(wo_hbm.at[r, :], wo_v.at[r, :], head_sems.at[2])

        def tail_copy(item):
            which, r, s = item
            if which is not None:
                return kv_copy(jnp.int32(NB // _PAIRS - 1), which, r, tail_sems.at[s])
            r = pl.ds(r, _WO_ROWS)
            return pltpu.make_async_copy(wo_hbm.at[r, :], wo_v.at[r, :], tail_sems.at[s])

        def request(lo_copy, hi_copy, first, last):
            for i0 in range(first, last, _GROUP):
                for i in range(i0, i0 + _GROUP):
                    lo_copy(i).start(priority=1)
                for i in range(i0, i0 + _GROUP):
                    hi_copy(i - _HALF).start(priority=0)

        def request_first_half(n, by_pair, prev_by_pair):
            prev = block_copies(n - 1, 1, prev_by_pair)
            request(block_copies(n, 0, by_pair), lambda i: prev(NP + i), 0, _HALF)

        def request_second_half(n, by_pair):
            request(block_copies(n, 0, by_pair), block_copies(n, 1, by_pair), _HALF, NP)

        def wait_for(ref, sem):
            pltpu.make_async_copy(ref, ref, sem).wait()

        x_copy = pltpu.make_async_copy(x_hbm, x_v, head_sems.at[0])
        x_copy.start()
        for k in range(_HALF):
            wq_copy(jnp.int32(k)).start(priority=1)

        @pl.loop(_HALF, NQ - NW + _HALF, step=_GROUP)
        def _(k):
            request(lambda i: wq_copy(k + i), lambda i: wq_copy(NW + k + i), 0, _GROUP)

        @pl.loop(NQ - NW + _HALF, NW, step=_GROUP)
        def _(k):
            request(lambda i: wq_copy(k + i), lambda i: wo_copy(NW - NQ + k + i), 0, _GROUP)

        request(block_copies(jnp.int32(0), 0, False),
                lambda i: wo_copy(jnp.int32(NO + i)), 0, _HALF)

        @pl.loop(0, _PAIRS)
        def _(n):
            request_second_half(n, False)
            request_first_half(n + 1, False, False)

        x_copy.wait()
        for b in range(B):
            xb = x_v[b].astype(jnp.float32)
            x_dup[pl.ds(8 * b, SQ), :] = xb
            x_dup[pl.ds(8 * b + SQ, SQ), :] = xb
        acc[...] = jnp.zeros_like(acc)
        wait_for(wq_v, head_sems.at[1])
        wait_for(wo_v.at[pl.ds(0, r_last)], head_sems.at[2])

        first8 = lax.broadcasted_iota(jnp.int32, (8, 1), 0) < SQ
        first_all = (lax.broadcasted_iota(jnp.int32, (8 * B, 1), 0) & SQ) == 0

        def tile(slot, which, row, n=DH):
            return kv[slot, which, pl.ds(row, n), :]

        def softmax_terms(slot, p, b, t):
            q = q_scr[p, pl.ds(pl.multiple_of(b * 8, 8), 8), :].astype(cdt)
            s = jnp.where(first8, _dot(q, tile(slot, 0, t)), _dot(q, tile(slot, 0, t + DH)))
            s = s * scale
            e = jnp.exp(s - jnp.max(s, axis=1, keepdims=True))
            return e.astype(cdt), jnp.sum(e, axis=1, keepdims=True)

        def wo_rows(row, n=DH):
            return wo_v[pl.ds(row, n), :]

        @pl.loop(0, NB - 1)
        def _(n):
            u, p = lax.div(n, _PAIRS), lax.rem(n, _PAIRS)
            slot, b = lax.rem(u, 3), lax.rem(u, B)
            t = pl.multiple_of(p * PAIR, PAIR)
            w = pl.multiple_of((lax.div(u, B) * _PAIRS + p) * PAIR, PAIR)

            n0 = N_MAIN - _PAIRS
            h0 = jnp.where(n <= n0, 2 * (n + _PAIRS) + 1, 2 * N_MAIN + 2 + n - n0)
            h1 = jnp.where(n <= n0, h0 + 1, h0)
            h_pair, h_tail = 2 * N_MAIN, 2 * (NB - 1)

            @pl.when(h0 < h_pair)
            def _():
                request_second_half(lax.div(h0, 2), False)

            @pl.when((lax.rem(h0, 2) == 1) & (h0 > h_pair) & (h0 < h_tail))
            def _():
                request_second_half(lax.div(h0, 2), True)

            @pl.when(h1 < h_pair)
            def _():
                request_first_half(lax.div(h1, 2), False, False)

            @pl.when(h1 == h_pair)
            def _():
                request_first_half(jnp.int32(N_MAIN), True, False)

            @pl.when((lax.rem(h1, 2) == 0) & (h1 > h_pair) & (h1 < h_tail))
            def _():
                request_first_half(lax.div(h1, 2), True, True)

            @pl.when(h1 == h_tail)
            def _():
                prev = block_copies(jnp.int32(NB - 2), 1, True)
                request(lambda i: tail_copy(tail_lo[i]), lambda i: prev(NP + i), 0, _HALF)

            for c in (1, 2):
                @pl.when(h1 == h_tail + c)
                def _():
                    request(lambda i: tail_copy(tail_lo[i]), lambda i: tail_copy(tail_hi[i]),
                            c * _HALF, (c + 1) * _HALF)

            @pl.when(b == 0)
            def _():
                q = _dot(x_dup[...].astype(wq_v.dtype), wq_v[:, pl.ds(w, PAIR)])
                q_scr[p] = jnp.where(first_all, q[:, :DH], q[:, DH:])

            @pl.when((p == 0) & (n < N_MAIN))
            def _():
                wait_for(kv.at[slot], unit_sems.at[slot])

            @pl.when(n >= N_MAIN)
            def _():
                wait_for(kv.at[slot, :, pl.ds(t, PAIR)], pair_sems.at[p])

            e, denom = softmax_terms(slot, p, b, t)
            o = jnp.where(first8, _dot_nt(e, tile(slot, 1, t)), _dot_nt(e, tile(slot, 1, t + DH)))
            o_scr[p, pl.ds(pl.multiple_of(b * 8, 8), 8), :] = o / denom

            @pl.when(b == B - 1)
            def _():
                o_all = o_scr[p]
                acc[...] += (
                    _dot(jnp.where(first_all, o_all, 0.0).astype(wo_v.dtype), wo_rows(w))
                    + _dot(jnp.where(first_all, 0.0, o_all).astype(wo_v.dtype), wo_rows(w + DH)))

        slot, p, rows = (NB // _PAIRS - 1) % 3, _PAIRS - 1, pl.ds(8 * (B - 1), 8)
        lo, hi = pl.ds(0, 128), pl.ds(128, DH - 128)

        wait_for(kv.at[slot, 0, pl.ds(t_last, PAIR)], tail_sems.at[0])
        e, denom = softmax_terms(slot, p, jnp.int32(B - 1), t_last)
        wait_for(kv.at[slot, 1, pl.ds(t_last, DH)], tail_sems.at[1])
        o_first = _dot_nt(e, tile(slot, 1, t_last))
        wait_for(kv.at[slot, 1, pl.ds(t_last + DH, 128)], tail_sems.at[2])
        o_lo = _dot_nt(e, tile(slot, 1, t_last + DH, 128))
        o_scr[p, rows, lo] = jnp.where(first8, o_first[:, :128], o_lo) / denom
        wait_for(kv.at[slot, 1, pl.ds(t_last + DH + 128, DH - 128)], tail_sems.at[3])
        o_hi = _dot_nt(e, tile(slot, 1, t_last + DH + 128, DH - 128))
        o_scr[p, rows, hi] = jnp.where(first8, o_first[:, 128:], o_hi) / denom

        wait_for(wo_v.at[pl.ds(r_last, DH)], tail_sems.at[4])
        res = acc[...] + _dot(
            jnp.where(first_all, o_scr[p], 0.0).astype(wo_v.dtype), wo_rows(r_last))
        wait_for(wo_v.at[pl.ds(r_last + DH, 128)], tail_sems.at[5])
        res += _dot(jnp.where(first_all, 0.0, o_scr[p, :, lo]).astype(wo_v.dtype),
                    wo_rows(r_last + DH, 128))
        wait_for(wo_v.at[pl.ds(r_last + DH + 128, DH - 128)], tail_sems.at[6])
        res += _dot(jnp.where(first_all, 0.0, o_scr[p, :, hi]).astype(wo_v.dtype),
                    wo_rows(r_last + DH + 128, DH - 128))
        for b in range(B):
            o_ref[b] = (res[8 * b:8 * b + SQ] + res[8 * b + SQ:8 * b + 8]).astype(o_ref.dtype)

    k_t = jnp.swapaxes(k_cache, 2, 3).reshape(B * H * DH, SK)
    v_t = jnp.swapaxes(v_cache, 2, 3).reshape(B * H * DH, SK)
    return pl.pallas_call(
        kernel,
        in_specs=[pl.BlockSpec(memory_space=pl.ANY)] * 5,
        out_specs=pl.BlockSpec(memory_space=pltpu.VMEM),
        out_shape=jax.ShapeDtypeStruct((B, SQ, D), x.dtype),
        scratch_shapes=[
            pltpu.VMEM((3, 2, UNIT, W), cdt),
            pltpu.VMEM(wq.shape, wq.dtype),
            pltpu.VMEM(wo.shape, wo.dtype),
            pltpu.VMEM(x.shape, x.dtype),
            pltpu.VMEM((8 * B, D), jnp.float32),
            pltpu.VMEM((_PAIRS, 8 * B, DH), jnp.float32),
            pltpu.VMEM((_PAIRS, 8 * B, DH), jnp.float32),
            pltpu.VMEM((8 * B, D), jnp.float32),
            pltpu.SemaphoreType.DMA((3,)),
            pltpu.SemaphoreType.DMA((3,)),
            pltpu.SemaphoreType.DMA((_PAIRS,)),
            pltpu.SemaphoreType.DMA((7,)),
        ],
        compiler_params=pltpu.CompilerParams(
            vmem_limit_bytes=64 * 1024 * 1024,
            disable_bounds_checks=True,
        ),
    )(x, k_t, v_t, wq, wo)
```

```python
import jax
import jax.numpy as jnp
from jax import lax
import jax.experimental.pallas as pl
import jax.experimental.pallas.tpu as pltpu

_HEADS = 32
_ROWS = 8
_REGION = 64
_PAIRS = 4
_GROUP = 2
_HALF = 24
_WQ_COLS = 1024
_WO_ROWS = 16
_WQ_SPREAD, _WO_SPREAD = 8, 6
_GRAY = (0, 1, 3, 2, 6, 7, 5, 4)
_NT = (((1,), (1,)), ((), ()))


def _dot(a, b):
    return jnp.dot(a, b, preferred_element_type=jnp.float32)


def _dot_nt(a, b):
    return lax.dot_general(a, b, _NT, preferred_element_type=jnp.float32)


@jax.jit
def pallas_standalone__sliding_block_cached__sampling_kernel(
    x: jax.Array,
    k_cache: jax.Array,
    v_cache: jax.Array,
    wq: jax.Array,
    wo: jax.Array,
):
    B, SQ, D = x.shape
    _, H, SK, DH = k_cache.shape
    W = min(4096, max(256, SK // 4))
    scale = DH**-0.5
    cdt = k_cache.dtype

    PAIR = 2 * DH
    UNIT = _PAIRS * PAIR
    NB = B * H // 2
    N_MAIN = NB - _PAIRS
    NP = 2 * _HALF
    NR = UNIT // _REGION
    assert (H, SQ, DH, _PAIRS) == (_HEADS, 4, 3 * _REGION, 4) and NP * _ROWS == PAIR

    regions = list(range(0, NR, 2)) + list(range(1, NR, 2))
    groups = [_ROWS * g for g in _GRAY]

    r_last = (H - 2) * DH
    n_wq_cols = H * DH // _WQ_COLS
    NQ = (D // 8) * n_wq_cols
    NO = r_last // _WO_ROWS
    NW = (NQ + NO) // 2
    assert D % 8 == 0 and n_wq_cols * _WQ_COLS == H * DH and NO * _WO_ROWS == r_last
    assert NQ % _WQ_SPREAD == 0 and NO % _WO_SPREAD == 0
    assert NW <= NQ < 2 * NW - _HALF and NQ % _GROUP == 0 and NW % _GROUP == 0

    t_last = UNIT - PAIR
    tail = [(0, t_last + r * _REGION + g, 0) for g in groups for r in range(6)]
    tail += [(1, t_last + r * _REGION + g, 1) for g in groups for r in range(3)]
    tail += [(1, t_last + r * _REGION + g, 2) for g in groups for r in range(3, 5)]
    tail += [(1, t_last + 5 * _REGION + g, 3) for g in groups]
    tail += [(None, r, 4) for r in range(r_last, r_last + DH, _WO_ROWS)]
    tail += [(None, r, 5) for r in range(r_last + DH, r_last + DH + 128, _WO_ROWS)]
    tail += [(None, r, 6) for r in range(r_last + DH + 128, H * DH, _WO_ROWS)]
    n_both = len(tail) - _HALF
    assert n_both == 2 * NP
    tail_lo = [c for i, c in enumerate(tail[:n_both]) if (i // _GROUP) % 2 == 0]
    tail_lo += tail[n_both:]
    tail_hi = [c for i, c in enumerate(tail[:n_both]) if (i // _GROUP) % 2 == 1]

    def kernel(x_hbm, k_hbm, v_hbm, wq_hbm, wo_hbm, o_ref,
               kv, wq_v, wo_v, x_v, x_dup, q_scr, o_scr, acc,
               unit_sems, head_sems, pair_sems, tail_sems):
        def kv_copy(u, which, r, sem):
            row = (lax.rem(u, B) * H + lax.div(u, B) * 2 * _PAIRS) * DH + r
            src = (k_hbm, v_hbm)[which]
            return pltpu.make_async_copy(
                src.at[pl.ds(pl.multiple_of(row, _ROWS), _ROWS), pl.ds(SK - W, W)],
                kv.at[lax.rem(u, 3), which, pl.ds(pl.multiple_of(r, _ROWS), _ROWS), :],
                sem,
            )

        def block_copies(n, which, by_pair):
            u, p = lax.div(n, _PAIRS), lax.rem(n, _PAIRS)
            if by_pair:
                return lambda i: kv_copy(
                    u, which, p * PAIR + ((i % 6) * _REGION + groups[i // 6]), pair_sems.at[p])
            gs = [(s ^ (s >> 1)) * _ROWS for s in (2 * p, 2 * p + 1)]
            return lambda i: kv_copy(
                u, which, regions[i % NR] * _REGION + gs[i // NR], unit_sems.at[lax.rem(u, 3)])

        def wq_copy(k):
            idx = lax.rem(k, _WQ_SPREAD) * (NQ // _WQ_SPREAD) + lax.div(k, _WQ_SPREAD)
            r = pl.ds(pl.multiple_of(lax.div(idx, n_wq_cols) * 8, 8), 8)
            c = pl.ds(pl.multiple_of(lax.rem(idx, n_wq_cols) * _WQ_COLS, _WQ_COLS), _WQ_COLS)
            return pltpu.make_async_copy(wq_hbm.at[r, c], wq_v.at[r, c], head_sems.at[1])

        def wo_copy(k):
            idx = lax.rem(k, _WO_SPREAD) * (NO // _WO_SPREAD) + lax.div(k, _WO_SPREAD)
            r = pl.ds(pl.multiple_of(idx * _WO_ROWS, _WO_ROWS), _WO_ROWS)
            return pltpu.make_async_copy(wo_hbm.at[r, :], wo_v.at[r, :], head_sems.at[2])

        def tail_copy(item):
            which, r, s = item
            if which is not None:
                return kv_copy(jnp.int32(NB // _PAIRS - 1), which, jnp.int32(r), tail_sems.at[s])
            r = pl.ds(r, _WO_ROWS)
            return pltpu.make_async_copy(wo_hbm.at[r, :], wo_v.at[r, :], tail_sems.at[s])

        def request(lo_copy, hi_copy, first, last):
            for i0 in range(first, last, _GROUP):
                for i in range(i0, i0 + _GROUP):
                    lo_copy(i).start(priority=1)
                for i in range(i0, i0 + _GROUP):
                    hi_copy(i - _HALF).start(priority=0)

        def request_first_half(n, by_pair, prev_by_pair):
            prev = block_copies(n - 1, 1, prev_by_pair)
            request(block_copies(n, 0, by_pair), lambda i: prev(NP + i), 0, _HALF)

        def request_second_half(n, by_pair):
            request(block_copies(n, 0, by_pair), block_copies(n, 1, by_pair), _HALF, NP)

        def wait_for(ref, sem):
            pltpu.make_async_copy(ref, ref, sem).wait()

        x_copy = pltpu.make_async_copy(x_hbm, x_v, head_sems.at[0])
        x_copy.start()
        for k in range(_HALF):
            wq_copy(jnp.int32(k)).start(priority=1)

        @pl.loop(_HALF, NQ - NW + _HALF, step=_GROUP)
        def _(k):
            request(lambda i: wq_copy(k + i), lambda i: wq_copy(NW + k + i), 0, _GROUP)

        @pl.loop(NQ - NW + _HALF, NW, step=_GROUP)
        def _(k):
            request(lambda i: wq_copy(k + i), lambda i: wo_copy(NW - NQ + k + i), 0, _GROUP)

        request(block_copies(jnp.int32(0), 0, False),
                lambda i: wo_copy(jnp.int32(NO + i)), 0, _HALF)

        @pl.loop(0, _PAIRS)
        def _(n):
            request_second_half(n, False)
            request_first_half(n + 1, False, False)

        x_copy.wait()
        for b in range(B):
            xb = x_v[b].astype(jnp.float32)
            x_dup[pl.ds(8 * b, SQ), :] = xb
            x_dup[pl.ds(8 * b + SQ, SQ), :] = xb
        acc[...] = jnp.zeros_like(acc)
        wait_for(wq_v, head_sems.at[1])
        wait_for(wo_v.at[pl.ds(0, r_last)], head_sems.at[2])

        first8 = lax.broadcasted_iota(jnp.int32, (8, 1), 0) < SQ
        first_all = (lax.broadcasted_iota(jnp.int32, (8 * B, 1), 0) & SQ) == 0

        def tile(slot, which, row, n=DH):
            return kv[slot, which, pl.ds(row, n), :]

        def softmax_terms(slot, p, b, t):
            q = q_scr[p, pl.ds(pl.multiple_of(b * 8, 8), 8), :].astype(cdt)
            s = jnp.where(first8, _dot(q, tile(slot, 0, t)), _dot(q, tile(slot, 0, t + DH)))
            s = s * scale
            e = jnp.exp(s - jnp.max(s, axis=1, keepdims=True))
            return e.astype(cdt), jnp.sum(e, axis=1, keepdims=True)

        def wo_rows(row, n=DH):
            return wo_v[pl.ds(row, n), :]

        @pl.loop(0, NB - 1)
        def _(n):
            u, p = lax.div(n, _PAIRS), lax.rem(n, _PAIRS)
            slot, b = lax.rem(u, 3), lax.rem(u, B)
            t = pl.multiple_of(p * PAIR, PAIR)
            w = pl.multiple_of((lax.div(u, B) * _PAIRS + p) * PAIR, PAIR)

            left = N_MAIN - n

            @pl.when(left > 4)
            def _():
                request_second_half(n + 4, False)

            @pl.when(left > 5)
            def _():
                request_first_half(n + 5, False, False)

            @pl.when(left == 5)
            def _():
                request_first_half(jnp.int32(N_MAIN), True, False)

            @pl.when((left == 4) | (left == 3) | (left == 0))
            def _():
                request_second_half(jnp.minimum(n + 4, N_MAIN + 2), True)

            @pl.when((left == 4) | (left == 2))
            def _():
                request_first_half(jnp.minimum(n + 5, N_MAIN + 2), True, True)

            @pl.when(left == -1)
            def _():
                prev = block_copies(jnp.int32(NB - 2), 1, True)
                request(lambda i: tail_copy(tail_lo[i]), lambda i: prev(NP + i), 0, _HALF)

            @pl.when(left == -2)
            def _():
                request(lambda i: tail_copy(tail_lo[i]), lambda i: tail_copy(tail_hi[i]),
                        _HALF, NP)

            @pl.when(b == 0)
            def _():
                q = _dot(x_dup[...].astype(wq_v.dtype), wq_v[:, pl.ds(w, PAIR)])
                q_scr[p] = jnp.where(first_all, q[:, :DH], q[:, DH:])

            @pl.when((p == 0) & (n < N_MAIN))
            def _():
                wait_for(kv.at[slot], unit_sems.at[slot])

            @pl.when(n >= N_MAIN)
            def _():
                wait_for(kv.at[slot, :, pl.ds(t, PAIR)], pair_sems.at[p])

            e, denom = softmax_terms(slot, p, b, t)
            o = jnp.where(first8, _dot_nt(e, tile(slot, 1, t)), _dot_nt(e, tile(slot, 1, t + DH)))
            o_scr[p, pl.ds(pl.multiple_of(b * 8, 8), 8), :] = o / denom

            @pl.when(b == B - 1)
            def _():
                o_all = o_scr[p]
                acc[...] += (
                    _dot(jnp.where(first_all, o_all, 0.0).astype(wo_v.dtype), wo_rows(w))
                    + _dot(jnp.where(first_all, 0.0, o_all).astype(wo_v.dtype), wo_rows(w + DH)))

        request(lambda i: tail_copy(tail_lo[i]), lambda i: tail_copy(tail_hi[i]),
                NP, len(tail_lo))
        slot, p, rows = (NB // _PAIRS - 1) % 3, _PAIRS - 1, pl.ds(8 * (B - 1), 8)
        lo, hi = pl.ds(0, 128), pl.ds(128, DH - 128)

        wait_for(kv.at[slot, 0, pl.ds(t_last, PAIR)], tail_sems.at[0])
        e, denom = softmax_terms(slot, p, jnp.int32(B - 1), t_last)
        wait_for(kv.at[slot, 1, pl.ds(t_last, DH)], tail_sems.at[1])
        o_first = _dot_nt(e, tile(slot, 1, t_last))
        wait_for(kv.at[slot, 1, pl.ds(t_last + DH, 128)], tail_sems.at[2])
        o_lo = _dot_nt(e, tile(slot, 1, t_last + DH, 128))
        o_scr[p, rows, lo] = jnp.where(first8, o_first[:, :128], o_lo) / denom
        wait_for(kv.at[slot, 1, pl.ds(t_last + DH + 128, DH - 128)], tail_sems.at[3])
        o_hi = _dot_nt(e, tile(slot, 1, t_last + DH + 128, DH - 128))
        o_scr[p, rows, hi] = jnp.where(first8, o_first[:, 128:], o_hi) / denom

        wait_for(wo_v.at[pl.ds(r_last, DH)], tail_sems.at[4])
        res = acc[...] + _dot(
            jnp.where(first_all, o_scr[p], 0.0).astype(wo_v.dtype), wo_rows(r_last))
        wait_for(wo_v.at[pl.ds(r_last + DH, 128)], tail_sems.at[5])
        res += _dot(jnp.where(first_all, 0.0, o_scr[p, :, lo]).astype(wo_v.dtype),
                    wo_rows(r_last + DH, 128))
        wait_for(wo_v.at[pl.ds(r_last + DH + 128, DH - 128)], tail_sems.at[6])
        res += _dot(jnp.where(first_all, 0.0, o_scr[p, :, hi]).astype(wo_v.dtype),
                    wo_rows(r_last + DH + 128, DH - 128))
        for b in range(B):
            o_ref[b] = (res[8 * b:8 * b + SQ] + res[8 * b + SQ:8 * b + 8]).astype(o_ref.dtype)

    k_t = jnp.swapaxes(k_cache, 2, 3).reshape(B * H * DH, SK)
    v_t = jnp.swapaxes(v_cache, 2, 3).reshape(B * H * DH, SK)
    return pl.pallas_call(
        kernel,
        in_specs=[pl.BlockSpec(memory_space=pl.ANY)] * 5,
        out_specs=pl.BlockSpec(memory_space=pltpu.VMEM),
        out_shape=jax.ShapeDtypeStruct((B, SQ, D), x.dtype),
        scratch_shapes=[
            pltpu.VMEM((3, 2, UNIT, W), cdt),
            pltpu.VMEM(wq.shape, wq.dtype),
            pltpu.VMEM(wo.shape, wo.dtype),
            pltpu.VMEM(x.shape, x.dtype),
            pltpu.VMEM((8 * B, D), jnp.float32),
            pltpu.VMEM((_PAIRS, 8 * B, DH), jnp.float32),
            pltpu.VMEM((_PAIRS, 8 * B, DH), jnp.float32),
            pltpu.VMEM((8 * B, D), jnp.float32),
            pltpu.SemaphoreType.DMA((3,)),
            pltpu.SemaphoreType.DMA((3,)),
            pltpu.SemaphoreType.DMA((_PAIRS,)),
            pltpu.SemaphoreType.DMA((7,)),
        ],
        compiler_params=pltpu.CompilerParams(
            vmem_limit_bytes=64 * 1024 * 1024,
            disable_bounds_checks=True,
        ),
    )(x, k_t, v_t, wq, wo)
```
